```python
import os as _os
_os.environ.setdefault("JAX_PLATFORMS", "cpu")
import jax
import jax.numpy as jnp

def _softmax(x, axis=-1):
    return jax.nn.softmax(x, axis=axis)
def _gelu(x):
    return jax.nn.gelu(x, approximate=True)
def _silu(x):
    return jax.nn.silu(x)
def _sigmoid(x):
    return jax.nn.sigmoid(x)
def _layernorm(x, axis=-1, eps=1e-5):
    m = jnp.mean(x, axis=axis, keepdims=True)
    v = jnp.var(x, axis=axis, keepdims=True)
    return (x - m) / jnp.sqrt(v + eps)
def _scatter_add(tgt, idx, src, axis=0):
    return tgt.at[idx].add(src)
def _segment_sum(src, seg, n):
    return jax.ops.segment_sum(src, seg, n)
class _Rng:
    def __init__(self, key):
        self._k = key
    def _next(self):
        self._k, sub = jax.random.split(self._k)
        return sub
    def normal(self, shape):
        return jax.random.normal(self._next(), shape, dtype=jnp.bfloat16)
    def randint(self, lo, hi, shape):
        return jax.random.randint(self._next(), shape, lo, hi, dtype=jnp.int32)
    def uniform(self, shape, lo=0.0, hi=1.0):
        return jax.random.uniform(self._next(), shape, jnp.bfloat16, lo, hi)
    def permutation(self, n):
        return jax.random.permutation(self._next(), n)


kernel_name = 'standalone__dense_activation_silu__prompt'

def setup_inputs():
    _rng = _Rng(jax.random.key(int.from_bytes(__import__("os").urandom(4), "little")))
    _w = (lambda a: (lambda t: t.astype(jnp.bfloat16) if jnp.issubdtype(t.dtype, jnp.floating) else t)(jnp.asarray(a)))
    B, S, D, F = 1, 2048, 448, 1792
    return {
        "x": _w((lambda *s: _rng.normal(s) * 0.05)(B, S, D)),
        "w1": _w((lambda *s: _rng.normal(s) * 0.05)(D, F) * (D ** -0.5)),
        "w2": _w((lambda *s: _rng.normal(s) * 0.05)(F, D) * (F ** -0.5)),
    }

def reference(x, w1, w2):
    h = jnp.einsum("bsd,df->bsf", x, w1)
    h = _silu(h)
    out = jnp.einsum("bsf,fd->bsd", h, w2)
    return out
```

```python
import jax
import jax.numpy as jnp
import jax.experimental.pallas as pl
import jax.experimental.pallas.tpu as pltpu

U = 128


def _silu(h):
    t = 0.5 * h
    return t + t * jnp.tanh(t)


def _pack(v):
    return pltpu.bitcast(v, jnp.uint32)


def _unpack(v):
    return pltpu.bitcast(v, jnp.bfloat16)


@jax.jit
def pallas_standalone__dense_activation_silu__prompt_kernel(
    x: jax.Array,
    w1: jax.Array,
    w2: jax.Array,
):
    B, S, D = x.shape
    F = w1.shape[1]
    assert B == 1 and S == 2048 and D == 448 and F == 1792
    NX, NF = S // U, F // U

    stages = ((2, 2), (4, 3), (6, 6), (8, 14))
    m2_tiles = (4, 4)
    fused_tiles = (4, 2, 2)
    last_m2 = (1, 1)
    last_split = 7
    nsem = 2 * len(stages) + 2 + len(m2_tiles) + len(fused_tiles) + last_split

    def body(xt_hbm, w1_hbm, w2t_hbm, o_hbm, xv, w1v, w2v, w1t, hts, ov, sems):
        n = [0]

        def cp(src, dst, a, b):
            c = pltpu.make_async_copy(
                src.at[:, pl.ds(a * U, (b - a) * U)],
                dst.at[:, pl.ds(a * U, (b - a) * U)],
                sems.at[n[0]],
            )
            n[0] += 1
            return c

        copies = []
        px, pf = 0, 0
        for sx, sf in stages:
            copies.append([cp(w1_hbm, w1v, pf, sf), cp(xt_hbm, xv, px, sx)])
            px, pf = sx, sf
        copies.append([cp(w2t_hbm, w2v, 0, NF), cp(xt_hbm, xv, px, NX)])
        for cs in copies:
            for c in cs:
                c.start()

        def m1v(fa, fb, xa, xb):
            lhs = _unpack(w1t[pl.ds(fa * U // 2, (fb - fa) * U // 2), :])
            ht = jnp.dot(lhs, xv[:, pl.ds(xa * U, (xb - xa) * U)],
                         preferred_element_type=jnp.float32)
            return _silu(ht).astype(jnp.bfloat16)

        def m1(fa, fb, xa, xb):
            hts[pl.ds(fa * U // 2, (fb - fa) * U // 2),
                pl.ds(xa * U, (xb - xa) * U)] = _pack(m1v(fa, fb, xa, xb))

        def tr(fa, fb):
            w1t[pl.ds(fa * U // 2, (fb - fa) * U // 2), :] = _pack(
                w1v[:, pl.ds(fa * U, (fb - fa) * U)].T)

        px, pf = 0, 0
        for si, (sx, sf) in enumerate(stages):
            if si == 0:
                copies[0][0].wait()
                tr(0, sf)
                copies[0][1].wait()
                m1(0, sf, 0, sx)
            else:
                for c in copies[si]:
                    c.wait()
                m1(0, pf, px, sx)
                tr(pf, sf)
                m1(pf, sf, 0, sx)
            px, pf = sx, sf
        for c in copies[-1]:
            c.wait()

        outs = []

        def m2v(hb, a, b, split=1):
            o = jnp.dot(w2v[...], hb, preferred_element_type=jnp.float32).astype(jnp.bfloat16)
            nr = D // split
            for k in range(split):
                rows, cols = pl.ds(k * nr, nr), pl.ds(a * U, (b - a) * U)
                ov[rows, cols] = o[k * nr:(k + 1) * nr]
                c = pltpu.make_async_copy(ov.at[rows, cols], o_hbm.at[rows, cols], sems.at[n[0]])
                n[0] += 1
                c.start()
                outs.append(c)

        a = 0
        for t in m2_tiles:
            m2v(_unpack(hts[:, pl.ds(a * U, t * U)]), a, a + t)
            a += t
        for i, t in enumerate(fused_tiles):
            hb = m1v(0, NF, a, a + t)
            if i == len(fused_tiles) - 1:
                c0 = 0
                for j, tt in enumerate(last_m2):
                    m2v(hb[:, c0 * U:(c0 + tt) * U], a + c0, a + c0 + tt,
                        split=(last_split if j == len(last_m2) - 1 else 1))
                    c0 += tt
            else:
                m2v(hb, a, a + t)
            a += t
        for c in outs:
            c.wait()

    def kernel(*refs):
        @pl.when(pl.program_id(0) == 0)
        def _():
            body(*refs)

    xt = x.reshape(S, D).T
    w2t = w2.T
    out_t = pl.pallas_call(
        kernel,
        grid=(2,),
        in_specs=[pl.BlockSpec(memory_space=pl.ANY)] * 3,
        out_specs=pl.BlockSpec(memory_space=pl.ANY),
        out_shape=jax.ShapeDtypeStruct((D, S), x.dtype),
        scratch_shapes=[
            pltpu.VMEM((D, S), jnp.bfloat16),
            pltpu.VMEM((D, F), jnp.bfloat16),
            pltpu.VMEM((D, F), jnp.bfloat16),
            pltpu.VMEM((F // 2, D), jnp.uint32),
            pltpu.VMEM((F // 2, sum(m2_tiles) * U), jnp.uint32),
            pltpu.VMEM((D, S), jnp.bfloat16),
            pltpu.SemaphoreType.DMA((nsem,)),
        ],
        compiler_params=pltpu.CompilerParams(
            dimension_semantics=("arbitrary",),
            vmem_limit_bytes=100 * 1024 * 1024,
            disable_semaphore_checks=True,
            disable_bounds_checks=True,
        ),
    )(xt, w1, w2t)
    return out_t.T.reshape(B, S, D)
```

```python
import jax
import jax.numpy as jnp
from jax import lax
import jax.experimental.pallas as pl
import jax.experimental.pallas.tpu as pltpu

D, S, F = 448, 2048, 1792
U = 128
NX, NF = S // U, F // U
KB = (0, 128, 256, 384, 448)
NT = 4
P = 2

GS = (32, 32, 32, 36)
B1U, A1U = 6, 12
B2U, A2U = 12, 12
DEFER = 256
STEP2, STEP_M1, STEP_M2 = 8.3, 16.0, 7.75
TLAG, TSLOW, TRESUME = 24, 0.25, 1400
GUARD = 150
LASTROWS = 512
LAST_SPLIT = (128, 128, 96, 48, 32, 16)

G = max(GS)
FMT = tuple(F - 8 * g for g in GS)
FM = F - 8 * G
LOADS = (
    (("w1", 3, 4, 0, B1U),),
    (("x", 3, 4, 0, A1U),),
    (("x", 3, 4, A1U, NX), ("w1", 3, 4, B1U, NF), ("w1", 2, 3, 0, B2U), ("x", 2, 3, 0, A2U)),
    (("w1", 0, 2, 0, NF), ("w1", 2, 3, B2U, NF), ("x", 0, 2, 0, NX), ("x", 2, 3, A2U, NX),
     ("w2", 0, 4, 0, NF)),
)
N_IN = sum(len(ls) for ls in LOADS)
N_SEM = N_IN + NX - 1 + len(LAST_SPLIT)


def _silu(h):
    t = 0.5 * h
    return t + t * jnp.tanh(t)


def _pack(v):
    return pltpu.bitcast(v, jnp.uint32)


def _unpack(v):
    return pltpu.bitcast(v, jnp.bfloat16)


def _input_copies(xt_hbm, w1_hbm, w2t_hbm, xv, w1v, w2v, sems):
    arrs = dict(x=(xt_hbm, xv), w1=(w1_hbm, w1v), w2=(w2t_hbm, w2v))
    groups, n = [], 0
    for ls in LOADS:
        g = []
        for nm, k0, k1, a, b in ls:
            src, dst = arrs[nm]
            idx = (pl.ds(KB[k0], KB[k1] - KB[k0]), pl.ds(a * U, (b - a) * U))
            g.append(pltpu.make_async_copy(src.at[idx], dst.at[idx], sems.at[n]))
            n += 1
        groups.append(g)
    return groups


def _compute(groups, o_hbm, xv, w1v, w2v, w1t, hp, ov, xf, xb, wb, w2p, sems):
    B1, B2 = B1U * U, B2U * U
    never = pl.program_id(0) > 7
    never_w = jnp.broadcast_to(never, (P, 8, U))
    never_t = jnp.broadcast_to(never, (8 * P, 64))

    def wait(cs):
        for c in cs:
            c.wait()

    V = dict(gen=None, debt=0.0, last=None, count=0, tiles=0)

    def vpu_gen():
        order = [gi for g0 in range(G - 4, -1, -4) for gi in range(g0, g0 + 4, P)]
        tsteps = [(gi, k) for gi in order for k in range(64)]
        wf = _unpack(w1t[pl.ds(FM // 2, 4 * G), pl.ds(384, 64)]).astype(jnp.float32)
        tpos = [0, 0.0]

        def table(anchor):
            if tpos[0] >= GS[0] * 64 // P:
                tpos[1] += TSLOW if V["count"] >= TRESUME else 0.0
            else:
                tpos[1] += 1.0
            while tpos[0] < len(tsteps) and tpos[0] < tpos[1]:
                gi, k = tsteps[tpos[0]]
                tpos[0] += 1
                w = lax.select(never_t, jnp.concatenate([anchor[:, :64]] * P, axis=0),
                               wf[gi * 8:(gi + P) * 8])
                wb[k, pl.ds(gi, P)] = jnp.broadcast_to(w[:, k:k + 1], (8 * P, U)).reshape(P, 8, U)

        for _ in range(TLAG):
            table((yield))
        shape = (P, 4, 8, U)
        for tile in range(NT):
            a = 4 * tile
            for bi, gi in enumerate(order[:GS[tile] // P]):
                acc = None
                for k in range(64):
                    anchor = yield
                    V["count"] += 1
                    table(anchor)
                    assert bi * 64 + k < tpos[0]
                    ws = lax.select(never_w, lax.broadcast_in_dim(anchor, (P, 8, U), (1, 2)),
                                    wb[k, pl.ds(gi, P)])
                    if bi == 0 or tile == 0:
                        xs = jnp.stack([
                            jnp.broadcast_to(xf[pl.ds(k, 1), pl.ds((a + j) * U, U)], (8, U))
                            for j in range(4)])
                        if tile > 0:
                            xb[k] = xs
                    else:
                        xs = xb[k]
                    p = lax.mul(lax.broadcast_in_dim(ws, shape, (0, 2, 3)),
                                lax.broadcast_in_dim(xs, shape, (1, 2, 3)))
                    acc = p if acc is None else acc + p
                for i in range(P):
                    for j in range(4):
                        hp[pl.ds(FM + (gi + i) * 8, 8), pl.ds((a + j) * U, U)] = acc[i, j]
            V["tiles"] = tile + 1

    def vpu_send(anchor):
        try:
            V["gen"].send(anchor)
        except StopIteration:
            V["gen"] = None

    def track(r, rows, step, stop=None):
        V["last"] = r[rows - 8:rows, :U]
        t = V["debt"]
        while t < rows:
            if V["gen"] is not None and (stop is None or t < stop):
                i = min(int(t) // 8, rows // 8 - 1)
                vpu_send(r[i * 8:(i + 1) * 8, :U])
            t += step
        V["debt"] = max(t - rows, 0.0)

    def vpu_need(tile):
        while V["tiles"] <= tile:
            vpu_send(V["last"])

    def tr(k0, k1, fa, fb):
        ks = pl.ds(KB[k0], KB[k1] - KB[k0])
        w1t[pl.ds(fa * U // 2, (fb - fa) * U // 2), ks] = _pack(
            w1v[ks, pl.ds(fa * U, (fb - fa) * U)].T)

    def hidx(r0, r1, c0, c1):
        return (pl.ds(r0, r1 - r0), pl.ds(c0 * U, (c1 - c0) * U))

    def mm(k0, k1, r0, r1, c0, c1):
        ks = pl.ds(KB[k0], KB[k1] - KB[k0])
        lhs = _unpack(w1t[pl.ds(r0 // 2, (r1 - r0) // 2), ks])
        return jnp.dot(lhs, xv[ks, pl.ds(c0 * U, (c1 - c0) * U)],
                       preferred_element_type=jnp.float32)

    def part(k0, k1, r0, r1, c0, c1, step=None, acc=False, last=False):
        if r1 <= r0:
            return
        per = 4 // (k1 - k0)
        for j0 in range(c0, c1, per):
            r = mm(k0, k1, r0, r1, j0, j0 + per)
            if step:
                track(r, r1 - r0, step,
                      stop=(r1 - r0 - GUARD) if (last and j0 + per >= c1) else None)
            idx = hidx(r0, r1, j0, j0 + per)
            hp[idx] = r + hp[idx] if acc else r

    wait(groups[0])
    tr(3, 4, 0, B1U)
    wait(groups[1])
    part(3, 4, 0, B1, 0, A1U)

    wait(groups[2])
    part(3, 4, 0, B1, A1U, NX)
    tr(3, 4, B1U, NF)
    tr(2, 3, 0, B2U)
    xf[...] = xv[pl.ds(384, 64), :].astype(jnp.float32)
    V["gen"] = vpu_gen()
    next(V["gen"])
    part(2, 3, 0, B1, 0, A2U, STEP2, acc=True)
    k2hi = [min(B2, FMT[t]) if 4 * t < A2U else 0 for t in range(NT)]
    for t in range(NT):
        if 4 * t < A2U:
            part(2, 4, B1, k2hi[t], 4 * t, 4 * t + 4, STEP2)
    for t in range(NT):
        part(3, 4, max(k2hi[t], B1), FMT[t] - (DEFER if t == NT - 1 else 0), 4 * t, 4 * t + 4,
             STEP2, last=(t == NT - 1))

    wait(groups[3])
    part(3, 4, FMT[-1] - DEFER, FMT[-1], NX - 4, NX)
    tr(0, 2, 0, B2U)
    tr(0, 3, B2U, NF)
    w2p[...] = _pack(w2v[...])

    outs = []

    def store_out(o, c, pieces):
        r0 = 0
        for nr in pieces:
            idx = (pl.ds(r0, nr), pl.ds(c * U, U))
            ov[idx] = o[r0:r0 + nr]
            cp = pltpu.make_async_copy(ov.at[idx], o_hbm.at[idx], sems.at[N_IN + len(outs)])
            cp.start()
            outs.append(cp)
            r0 += nr

    def m2(c0, nc, rhs):
        p = jnp.dot(_unpack(w2p[:, pl.ds(c0, nc)]), rhs, preferred_element_type=jnp.float32)
        track(p, D, STEP_M2)
        return p

    for ti in range(NT):
        a = 4 * ti
        V["debt"] = 0.0
        cuts = sorted({0, k2hi[ti], F} | ({F - LASTROWS} if k2hi[ti] < F - LASTROWS else set()))
        pieces = []
        for r0, r1 in zip(cuts[:-1], cuts[1:]):
            nk = 2 if r1 <= k2hi[ti] else 3
            per = 2 if nk == 2 else 1
            if r1 > FMT[ti]:
                vpu_need(ti)
            rs = []
            for j0 in range(0, 4, per):
                r = mm(0, nk, r0, r1, a + j0, a + j0 + per)
                if nk == 2 or j0 < 3:
                    track(r, r1 - r0, STEP_M1)
                rs.append(_silu(r + hp[hidx(r0, r1, a + j0, a + j0 + per)]).astype(jnp.bfloat16))
            pieces.append(jnp.concatenate(rs, axis=1))
        hb = jnp.concatenate(pieces, axis=0)
        for c in (0, 2):
            tail = m2(1536, 256, hb[1536:, c * U:(c + 2) * U])
            for j in (c, c + 1):
                acc = tail[:, (j - c) * U:(j - c + 1) * U]
                for q in range(3):
                    acc = acc + m2(q * 512, 512, hb[q * 512:(q + 1) * 512, j * U:(j + 1) * U])
                store_out(acc.astype(jnp.bfloat16), a + j,
                          LAST_SPLIT if a + j == NX - 1 else (D,))
    assert V["gen"] is None and N_IN + len(outs) == N_SEM
    wait(outs)


def _kernel(xt_hbm, w1_hbm, w2t_hbm, o_hbm, xv, w1v, w2v, w1t, hp, ov, xf, xb, wb, w2p, sems):
    step = pl.program_id(0)

    @pl.when(step == 0)
    def _():
        for g in _input_copies(xt_hbm, w1_hbm, w2t_hbm, xv, w1v, w2v, sems):
            for c in g:
                c.start()

    @pl.when(step == 1)
    def _():
        groups = _input_copies(xt_hbm, w1_hbm, w2t_hbm, xv, w1v, w2v, sems)
        _compute(groups, o_hbm, xv, w1v, w2v, w1t, hp, ov, xf, xb, wb, w2p, sems)


@jax.jit
def pallas_standalone__dense_activation_silu__prompt_kernel(
    x: jax.Array,
    w1: jax.Array,
    w2: jax.Array,
):
    assert x.shape == (1, S, D) and w1.shape == (D, F) and w2.shape == (F, D)
    xt = x.reshape(S, D).T
    w2t = w2.T
    out_t = pl.pallas_call(
        _kernel,
        grid=(2,),
        in_specs=[pl.BlockSpec(memory_space=pl.ANY)] * 3,
        out_specs=pl.BlockSpec(memory_space=pl.ANY),
        out_shape=jax.ShapeDtypeStruct((D, S), x.dtype),
        scratch_shapes=[
            pltpu.VMEM((D, S), jnp.bfloat16),
            pltpu.VMEM((D, F), jnp.bfloat16),
            pltpu.VMEM((D, F), jnp.bfloat16),
            pltpu.VMEM((F // 2, D), jnp.uint32),
            pltpu.VMEM((F, S), jnp.float32),
            pltpu.VMEM((D, S), jnp.bfloat16),
            pltpu.VMEM((64, S), jnp.float32),
            pltpu.VMEM((64, 4, 8, U), jnp.float32),
            pltpu.VMEM((64, G, 8, U), jnp.float32),
            pltpu.VMEM((D // 2, F), jnp.uint32),
            pltpu.SemaphoreType.DMA((N_SEM,)),
        ],
        compiler_params=pltpu.CompilerParams(
            dimension_semantics=("arbitrary",),
            vmem_limit_bytes=100 * 1024 * 1024,
            disable_semaphore_checks=True,
            disable_bounds_checks=True,
        ),
    )(xt, w1, w2t)
    return out_t.T.reshape(1, S, D)
```

```python
import jax
import jax.numpy as jnp
from jax import lax
import jax.experimental.pallas as pl
import jax.experimental.pallas.tpu as pltpu

D, S, F = 448, 2048, 1792
U = 128
NX, NF = S // U, F // U
KB = (0, 128, 256, 384, 448)
NT = 4

G = 32
FM = F - 8 * G
P = 2
KS = 8
TLAG = 4
B1U, A1U = 6, 12
A2U = 12
B2U = FM // U
DEFER = 256
GUARD = 150
LASTROWS = 512
LAST_SPLIT = (128, 128, 96, 48, 32, 16)

LOADS = (
    (("w1", 3, 4, 0, B1U),),
    (("x", 3, 4, 0, A1U),),
    (("x", 3, 4, A1U, NX), ("w1", 3, 4, B1U, NF), ("w1", 2, 3, 0, B2U), ("x", 2, 3, 0, A2U)),
    (("w1", 0, 2, 0, NF), ("w1", 2, 3, B2U, NF), ("x", 0, 2, 0, NX), ("x", 2, 3, A2U, NX),
     ("w2", 0, 4, 0, NF)),
)
N_IN = sum(len(ls) for ls in LOADS)
N_SEM = N_IN + NX - 1 + len(LAST_SPLIT)


def _silu(h):
    t = 0.5 * h
    return t + t * jnp.tanh(t)


def _pack(v):
    return pltpu.bitcast(v, jnp.uint32)


def _unpack(v):
    return pltpu.bitcast(v, jnp.bfloat16)


def _input_copies(xt_hbm, w1_hbm, w2t_hbm, xv, w1v, w2v, sems):
    arrs = dict(x=(xt_hbm, xv), w1=(w1_hbm, w1v), w2=(w2t_hbm, w2v))
    groups, n = [], 0
    for ls in LOADS:
        g = []
        for nm, k0, k1, a, b in ls:
            src, dst = arrs[nm]
            idx = (pl.ds(KB[k0], KB[k1] - KB[k0]), pl.ds(a * U, (b - a) * U))
            g.append(pltpu.make_async_copy(src.at[idx], dst.at[idx], sems.at[n]))
            n += 1
        groups.append(g)
    return groups


def _compute(groups, o_hbm, xv, w1v, w2v, w1t, hp, ov, xf, xb, wb, w2p, sems):
    B1 = B1U * U
    never = pl.program_id(0) > 7
    never_w = jnp.broadcast_to(never, (KS, P, 8, U))
    never_x = jnp.broadcast_to(never, (KS, 4, 8, U))
    never_t = jnp.broadcast_to(never, (KS, P, 8, 64))

    def wait(cs):
        for c in cs:
            c.wait()

    V = dict(gen=None, debt=0, tiles=0)

    def to_f32(c0, c1):
        cs = pl.ds(c0 * U, (c1 - c0) * U)
        xf[:, cs] = xv[pl.ds(384, 64), cs].astype(jnp.float32)

    def x_rows(k0, a):
        return jnp.stack([
            jnp.broadcast_to(xf[pl.ds(k0 + kk, 1), pl.ds((a + j) * U, U)], (8, U))
            for kk in range(KS) for j in range(4)]).reshape(KS, 4, 8, U)

    def xb_gen():
        for k0 in range(0, 64, KS):
            anchor = yield
            xb[pl.ds(k0, KS)] = lax.select(
                never_x, lax.broadcast_in_dim(anchor, (KS, 4, 8, U), (0, 2, 3)), x_rows(k0, 0))

    def vpu_gen():
        order = list(range(G - P, -1, -P))
        tsteps = [(gi, k0) for gi in order for k0 in range(0, 64, KS)]
        wf = _unpack(w1t[pl.ds(FM // 2, 4 * G), pl.ds(384, 64)]).astype(jnp.float32)
        wf = wf.reshape(G, 8, 64)

        def table(anchor):
            if not tsteps:
                return
            gi, k0 = tsteps.pop(0)
            w = lax.select(
                never_t, lax.broadcast_in_dim(anchor[:, :, :64], (KS, P, 8, 64), (0, 2, 3)),
                lax.broadcast_in_dim(wf[gi:gi + P], (KS, P, 8, 64), (1, 2, 3)))
            for kk in range(KS):
                wb[pl.ds(k0 + kk, 1), pl.ds(gi, P)] = jnp.broadcast_to(
                    w[kk:kk + 1, :, :, k0 + kk:k0 + kk + 1], (1, P, 8, U))

        for _ in range(TLAG):
            table((yield))
        shape = (KS, P, 4, 8, U)
        for tile in range(NT):
            a = 4 * tile
            for bi, gi in enumerate(order):
                acc = None
                for k0 in range(0, 64, KS):
                    anchor = yield
                    table(anchor)
                    ws = lax.select(
                        never_w, lax.broadcast_in_dim(anchor, (KS, P, 8, U), (0, 2, 3)),
                        wb[pl.ds(k0, KS), pl.ds(gi, P)])
                    if bi == 0 and tile > 0:
                        xs = x_rows(k0, a)
                        xb[pl.ds(k0, KS)] = xs
                    else:
                        xs = xb[pl.ds(k0, KS)]
                    p = lax.mul(lax.broadcast_in_dim(ws, shape, (0, 1, 3, 4)),
                                lax.broadcast_in_dim(xs, shape, (0, 2, 3, 4)))
                    for kk in range(KS):
                        acc = p[kk:kk + 1] if acc is None else acc + p[kk:kk + 1]
                for i in range(P):
                    for j in range(4):
                        hp[pl.ds(FM + (gi + i) * 8, 8), pl.ds((a + j) * U, U)] = acc[0, i, j]
            V["tiles"] = tile + 1

    def start(gen):
        assert V["gen"] is None
        V["gen"], V["debt"] = gen, 0
        next(gen)

    def track(r, rows, step, stop=None):
        ng = rows // step
        r3 = r[:, :U].reshape(ng, step, U)
        if step > 8:
            r3 = r3[:, :8]
        t = V["debt"]
        while t < rows:
            if V["gen"] is not None and (stop is None or t < stop):
                i = min(t // step, ng - KS)
                try:
                    V["gen"].send(r3[i:i + KS])
                except StopIteration:
                    V["gen"] = None
            t += step * KS
        V["debt"] = t - rows

    def tr(k0, k1, fa, fb):
        ks = pl.ds(KB[k0], KB[k1] - KB[k0])
        w1t[pl.ds(fa * U // 2, (fb - fa) * U // 2), ks] = _pack(
            w1v[ks, pl.ds(fa * U, (fb - fa) * U)].T)

    def hidx(r0, r1, c0, c1):
        return (pl.ds(r0, r1 - r0), pl.ds(c0 * U, (c1 - c0) * U))

    def mm(k0, k1, r0, r1, c0, c1):
        ks = pl.ds(KB[k0], KB[k1] - KB[k0])
        lhs = _unpack(w1t[pl.ds(r0 // 2, (r1 - r0) // 2), ks])
        return jnp.dot(lhs, xv[ks, pl.ds(c0 * U, (c1 - c0) * U)],
                       preferred_element_type=jnp.float32)

    def part(k0, k1, r0, r1, c0, c1, step=None, acc=False, last=False):
        per = 4 // (k1 - k0)
        for j0 in range(c0, c1, per):
            r = mm(k0, k1, r0, r1, j0, j0 + per)
            if step:
                track(r, r1 - r0, step,
                      stop=(r1 - r0 - GUARD) if (last and j0 + per >= c1) else None)
            idx = hidx(r0, r1, j0, j0 + per)
            hp[idx] = r + hp[idx] if acc else r

    wait(groups[0])
    tr(3, 4, 0, B1U)
    wait(groups[1])
    to_f32(0, 4)
    start(xb_gen())
    part(3, 4, 0, B1, 0, A1U, 32)

    wait(groups[2])
    part(3, 4, 0, B1, A1U, NX)
    tr(3, 4, B1U, NF)
    tr(2, 3, B1U, B2U)
    tr(2, 3, 0, B1U)
    to_f32(4, NX)
    start(vpu_gen())
    part(2, 3, 0, B1, 0, A2U, 8, acc=True)
    part(2, 4, B1, FM, 0, A2U, 8)
    part(3, 4, B1, FM - DEFER, A2U, NX, 8, last=True)

    wait(groups[3])
    part(3, 4, FM - DEFER, FM, A2U, NX)
    tr(0, 2, 0, B2U)
    tr(0, 3, B2U, NF)
    w2p[...] = _pack(w2v[...])

    outs = []

    def store_out(o, c, pieces):
        r0 = 0
        for nr in pieces:
            idx = (pl.ds(r0, nr), pl.ds(c * U, U))
            ov[idx] = o[r0:r0 + nr]
            cp = pltpu.make_async_copy(ov.at[idx], o_hbm.at[idx], sems.at[N_IN + len(outs)])
            cp.start()
            outs.append(cp)
            r0 += nr

    def m2(c0, nc, rhs):
        p = jnp.dot(_unpack(w2p[:, pl.ds(c0, nc)]), rhs, preferred_element_type=jnp.float32)
        track(p, D, 8)
        return p

    for ti in range(NT):
        a = 4 * ti
        V["debt"] = 0
        todo = ((0, FM, 2), (FM, F, 3)) if a < A2U else ((0, F - LASTROWS, 3), (F - LASTROWS, F, 3))
        pieces = []
        for r0, r1, nk in todo:
            per = 2 if nk == 2 else 1
            if r1 > FM:
                assert V["tiles"] > ti
            rs = []
            for j0 in range(0, 4, per):
                r = mm(0, nk, r0, r1, a + j0, a + j0 + per)
                if nk == 2 or j0 < 3:
                    track(r, r1 - r0, 16)
                rs.append(_silu(r + hp[hidx(r0, r1, a + j0, a + j0 + per)]).astype(jnp.bfloat16))
            pieces.append(jnp.concatenate(rs, axis=1))
        hb = jnp.concatenate(pieces, axis=0)
        for c in (0, 2):
            tail = m2(1536, 256, hb[1536:, c * U:(c + 2) * U])
            for j in (c, c + 1):
                acc = tail[:, (j - c) * U:(j - c + 1) * U]
                for q in range(3):
                    acc = acc + m2(q * 512, 512, hb[q * 512:(q + 1) * 512, j * U:(j + 1) * U])
                store_out(acc.astype(jnp.bfloat16), a + j,
                          LAST_SPLIT if a + j == NX - 1 else (D,))
    assert V["gen"] is None and N_IN + len(outs) == N_SEM
    wait(outs)


def _kernel(xt_hbm, w1_hbm, w2t_hbm, o_hbm, xv, w1v, w2v, w1t, hp, ov, xf, xb, wb, w2p, sems):
    step = pl.program_id(0)

    @pl.when(step == 0)
    def _():
        for g in _input_copies(xt_hbm, w1_hbm, w2t_hbm, xv, w1v, w2v, sems):
            for c in g:
                c.start()

    @pl.when(step == 1)
    def _():
        groups = _input_copies(xt_hbm, w1_hbm, w2t_hbm, xv, w1v, w2v, sems)
        _compute(groups, o_hbm, xv, w1v, w2v, w1t, hp, ov, xf, xb, wb, w2p, sems)


@jax.jit
def pallas_standalone__dense_activation_silu__prompt_kernel(
    x: jax.Array,
    w1: jax.Array,
    w2: jax.Array,
):
    assert x.shape == (1, S, D) and w1.shape == (D, F) and w2.shape == (F, D)
    xt = x.reshape(S, D).T
    w2t = w2.T
    out_t = pl.pallas_call(
        _kernel,
        grid=(2,),
        in_specs=[pl.BlockSpec(memory_space=pl.ANY)] * 3,
        out_specs=pl.BlockSpec(memory_space=pl.ANY),
        out_shape=jax.ShapeDtypeStruct((D, S), x.dtype),
        scratch_shapes=[
            pltpu.VMEM((D, S), jnp.bfloat16),
            pltpu.VMEM((D, F), jnp.bfloat16),
            pltpu.VMEM((D, F), jnp.bfloat16),
            pltpu.VMEM((F // 2, D), jnp.uint32),
            pltpu.VMEM((F, S), jnp.float32),
            pltpu.VMEM((D, S), jnp.bfloat16),
            pltpu.VMEM((64, S), jnp.float32),
            pltpu.VMEM((64, 4, 8, U), jnp.float32),
            pltpu.VMEM((64, G, 8, U), jnp.float32),
            pltpu.VMEM((D // 2, F), jnp.uint32),
            pltpu.SemaphoreType.DMA((N_SEM,)),
        ],
        compiler_params=pltpu.CompilerParams(
            dimension_semantics=("arbitrary",),
            vmem_limit_bytes=100 * 1024 * 1024,
            disable_semaphore_checks=True,
            disable_bounds_checks=True,
        ),
    )(xt, w1, w2t)
    return out_t.T.reshape(1, S, D)
```

```python
import jax
import jax.numpy as jnp
from jax import lax
import jax.experimental.pallas as pl
import jax.experimental.pallas.tpu as pltpu

D, S, F = 448, 2048, 1792
U = 128
NX, NF = S // U, F // U
KB = (0, 128, 256, 384, 448)
NT = 4

GS = (32, 32, 32, 50)
G = max(GS)
FMT = tuple(F - 8 * g for g in GS)
FM = F - 8 * G
P = 2
NLATE, PRE = 9, 9
KS = 8
TLAG = 4
B1U, A1U = 6, 12
B2U, A2U = 12, 12
DEFER = 256
GUARD = 150
LASTROWS = 640
LAST_SPLIT = (128, 128, 96, 48, 32, 16)

LOADS = (
    (("w1", 3, 4, 0, B1U),),
    (("x", 3, 4, 0, A1U),),
    (("x", 3, 4, A1U, NX), ("w1", 3, 4, B1U, NF), ("w1", 2, 3, 0, B2U), ("x", 2, 3, 0, A2U)),
    (("w1", 0, 2, 0, NF), ("w1", 2, 3, B2U, NF), ("x", 0, 2, 0, NX), ("x", 2, 3, A2U, NX),
     ("w2", 0, 4, 0, NF)),
)
N_IN = sum(len(ls) for ls in LOADS)
N_SEM = N_IN + NX - 1 + len(LAST_SPLIT)


def _silu(h):
    t = 0.5 * h
    return t + t * jnp.tanh(t)


def _pack(v):
    return pltpu.bitcast(v, jnp.uint32)


def _unpack(v):
    return pltpu.bitcast(v, jnp.bfloat16)


def _input_copies(xt_hbm, w1_hbm, w2t_hbm, xv, w1v, w2v, sems):
    arrs = dict(x=(xt_hbm, xv), w1=(w1_hbm, w1v), w2=(w2t_hbm, w2v))
    groups, n = [], 0
    for ls in LOADS:
        g = []
        for nm, k0, k1, a, b in ls:
            src, dst = arrs[nm]
            idx = (pl.ds(KB[k0], KB[k1] - KB[k0]), pl.ds(a * U, (b - a) * U))
            g.append(pltpu.make_async_copy(src.at[idx], dst.at[idx], sems.at[n]))
            n += 1
        groups.append(g)
    return groups


def _compute(groups, o_hbm, xv, w1v, w2v, w1t, hp, ov, xf, xb, wb, w2p, sems):
    B1, B2 = B1U * U, B2U * U
    assert FMT[:3] == (B2,) * 3 and A2U == NX - 4
    never = pl.program_id(0) > 7
    never_w = jnp.broadcast_to(never, (KS, P, 8, U))
    never_x = jnp.broadcast_to(never, (KS, 4, 8, U))
    never_t = jnp.broadcast_to(never, (KS, P, 8, 64))

    def wait(cs):
        for c in cs:
            c.wait()

    V = dict(gen=None, debt=0, blocks=(0, 0), m2=False)

    def to_f32(c0, c1):
        cs = pl.ds(c0 * U, (c1 - c0) * U)
        xf[:, cs] = xv[pl.ds(384, 64), cs].astype(jnp.float32)

    def x_rows(k0, a):
        return jnp.stack([
            jnp.broadcast_to(xf[pl.ds(k0 + kk, 1), pl.ds((a + j) * U, U)], (8, U))
            for kk in range(KS) for j in range(4)]).reshape(KS, 4, 8, U)

    def xb_gen():
        for k0 in range(0, 64, KS):
            anchor = yield
            xb[pl.ds(k0, KS)] = lax.select(
                never_x, lax.broadcast_in_dim(anchor, (KS, 4, 8, U), (0, 2, 3)), x_rows(k0, 0))

    def vpu_gen():
        order = list(range(G - P, -1, -P))
        tsteps = [(gi, k0) for gi in order for k0 in range(0, 64, KS)]
        wf = _unpack(w1t[pl.ds(FM // 2, 4 * G), pl.ds(384, 64)]).astype(jnp.float32)
        wf = wf.reshape(G, 8, 64)
        n_extra = (G - GS[0]) // P * (64 // KS)

        def table(anchor):
            if not tsteps or (len(tsteps) <= n_extra and V["m2"]):
                return
            gi, k0 = tsteps.pop(0)
            w = lax.select(
                never_t, lax.broadcast_in_dim(anchor[:, :, :64], (KS, P, 8, 64), (0, 2, 3)),
                lax.broadcast_in_dim(wf[gi:gi + P], (KS, P, 8, 64), (1, 2, 3)))
            for kk in range(KS):
                wb[pl.ds(k0 + kk, 1), pl.ds(gi, P)] = jnp.broadcast_to(
                    w[kk:kk + 1, :, :, k0 + kk:k0 + kk + 1], (1, P, 8, U))

        for _ in range(TLAG):
            table((yield))
        shape = (KS, P, 4, 8, U)
        for tile in range(NT):
            a = 4 * tile
            blocks = order[:GS[tile] // P]
            if tile == NT - 1:
                blocks = blocks[NLATE:] + blocks[:NLATE][::-1]
            for bi, gi in enumerate(blocks):
                acc = None
                for k0 in range(0, 64, KS):
                    anchor = yield
                    table(anchor)
                    assert (gi, k0) not in tsteps
                    ws = lax.select(
                        never_w, lax.broadcast_in_dim(anchor, (KS, P, 8, U), (0, 2, 3)),
                        wb[pl.ds(k0, KS), pl.ds(gi, P)])
                    if bi == 0 and tile > 0:
                        xs = x_rows(k0, a)
                        xb[pl.ds(k0, KS)] = xs
                    else:
                        xs = xb[pl.ds(k0, KS)]
                    p = lax.mul(lax.broadcast_in_dim(ws, shape, (0, 1, 3, 4)),
                                lax.broadcast_in_dim(xs, shape, (0, 2, 3, 4)))
                    for kk in range(KS):
                        acc = p[kk:kk + 1] if acc is None else acc + p[kk:kk + 1]
                for i in range(P):
                    for j in range(4):
                        hp[pl.ds(FM + (gi + i) * 8, 8), pl.ds((a + j) * U, U)] = acc[0, i, j]
                V["blocks"] = (tile, bi + 1)

    def start(gen):
        assert V["gen"] is None
        V["gen"], V["debt"] = gen, 0
        next(gen)

    def track(r, rows, step, stop=None):
        ng = rows // step
        r3 = r[:, :U].reshape(ng, step, U)
        if step > 8:
            r3 = r3[:, :8]
        t = V["debt"]
        while t < rows:
            if V["gen"] is not None and (stop is None or t < stop):
                i = min(t // step, ng - KS)
                try:
                    V["gen"].send(r3[i:i + KS])
                except StopIteration:
                    V["gen"] = None
            t += step * KS
        V["debt"] = t - rows

    def tr(k0, k1, fa, fb):
        ks = pl.ds(KB[k0], KB[k1] - KB[k0])
        w1t[pl.ds(fa * U // 2, (fb - fa) * U // 2), ks] = _pack(
            w1v[ks, pl.ds(fa * U, (fb - fa) * U)].T)

    def hidx(r0, r1, c0, c1):
        return (pl.ds(r0, r1 - r0), pl.ds(c0 * U, (c1 - c0) * U))

    def mm(k0, k1, r0, r1, c0, c1):
        ks = pl.ds(KB[k0], KB[k1] - KB[k0])
        lhs = _unpack(w1t[pl.ds(r0 // 2, (r1 - r0) // 2), ks])
        return jnp.dot(lhs, xv[ks, pl.ds(c0 * U, (c1 - c0) * U)],
                       preferred_element_type=jnp.float32)

    def part(k0, k1, r0, r1, c0, c1, step=None, acc=False, last=False):
        per = 4 // (k1 - k0)
        for j0 in range(c0, c1, per):
            r = mm(k0, k1, r0, r1, j0, j0 + per)
            if step:
                track(r, r1 - r0, step,
                      stop=(r1 - r0 - GUARD) if (last and j0 + per >= c1) else None)
            idx = hidx(r0, r1, j0, j0 + per)
            hp[idx] = r + hp[idx] if acc else r

    wait(groups[0])
    tr(3, 4, 0, B1U)
    wait(groups[1])
    to_f32(0, 4)
    start(xb_gen())
    part(3, 4, 0, B1, 0, A1U, 32)

    wait(groups[2])
    part(3, 4, 0, B1, A1U, NX)
    tr(3, 4, B1U, NF)
    tr(2, 3, B1U, B2U)
    tr(2, 3, 0, B1U)
    to_f32(4, NX)
    start(vpu_gen())
    part(2, 3, 0, B1, 0, A2U, 8, acc=True)
    part(2, 4, B1, B2, 0, A2U, 8)
    part(3, 4, B1, FMT[-1] - DEFER, A2U, NX, 8, last=True)

    wait(groups[3])
    part(3, 4, FMT[-1] - DEFER, FMT[-1], A2U, NX)
    tr(0, 2, 0, B2U)
    tr(0, 3, B2U, NF)
    w2p[...] = _pack(w2v[...])

    outs = []

    def store_out(o, c, pieces):
        r0 = 0
        for nr in pieces:
            idx = (pl.ds(r0, nr), pl.ds(c * U, U))
            ov[idx] = o[r0:r0 + nr]
            cp = pltpu.make_async_copy(ov.at[idx], o_hbm.at[idx], sems.at[N_IN + len(outs)])
            cp.start()
            outs.append(cp)
            r0 += nr

    def m2(c0, nc, rhs):
        p = jnp.dot(_unpack(w2p[:, pl.ds(c0, nc)]), rhs, preferred_element_type=jnp.float32)
        V["m2"] = True
        track(p, D, 8)
        V["m2"] = False
        return p

    for ti in range(NT):
        a = 4 * ti
        last = ti == NT - 1
        V["debt"] = 0
        todo = ((0, F - LASTROWS, 3), (F - LASTROWS, F, 3)) if last else ((0, B2, 2), (B2, F, 3))
        l0 = F - 8 * P * NLATE if last else F
        pieces, raws = [], []
        for r0, r1, nk in todo:
            per = 2 if nk == 2 else 1
            rm = min(r1, l0)
            if r1 > FMT[ti]:
                assert V["blocks"] >= (ti, GS[ti] // P - (NLATE if last else 0))
            rs = []
            for j0 in range(0, 4, per):
                r = mm(0, nk, r0, r1, a + j0, a + j0 + per)
                if nk == 2 or j0 < 3:
                    track(r, r1 - r0, 16)
                rs.append(_silu(r[:rm - r0] + hp[hidx(r0, rm, a + j0, a + j0 + per)])
                          .astype(jnp.bfloat16))
                if rm < r1:
                    raws.append(r[rm - r0:])
            pieces.append(jnp.concatenate(rs, axis=1))
        hb = jnp.concatenate(pieces, axis=0)
        if not last:
            for c in (0, 2):
                tail = m2(1536, 256, hb[1536:, c * U:(c + 2) * U])
                for j in (c, c + 1):
                    acc = tail[:, (j - c) * U:(j - c + 1) * U]
                    for q in range(3):
                        acc = acc + m2(q * 512, 512, hb[q * 512:(q + 1) * 512, j * U:(j + 1) * U])
                    store_out(acc.astype(jnp.bfloat16), a + j, (D,))
            continue
        assert PRE == 9
        accs = [None] * 4
        for idx in range(12):
            j, q = divmod(idx, 3)
            if idx == PRE:
                assert V["gen"] is None
                for c in (0, 2):
                    cols = []
                    for jj in (c, c + 1):
                        hl = _silu(raws[jj] + hp[hidx(l0, F, a + jj, a + jj + 1)])
                        cols.append(jnp.concatenate(
                            [hb[1536:l0, jj * U:(jj + 1) * U], hl.astype(jnp.bfloat16)], axis=0))
                    tail = m2(1536, 256, jnp.concatenate(cols, axis=1))
                    for jj in (c, c + 1):
                        pj = tail[:, (jj - c) * U:(jj - c + 1) * U]
                        accs[jj] = pj if accs[jj] is None else accs[jj] + pj
                for jj in range(3):
                    store_out(accs[jj].astype(jnp.bfloat16), a + jj, (D,))
            p = m2(q * 512, 512, hb[q * 512:(q + 1) * 512, j * U:(j + 1) * U])
            accs[j] = p if accs[j] is None else accs[j] + p
        store_out(accs[3].astype(jnp.bfloat16), a + 3, LAST_SPLIT)
    assert V["gen"] is None and N_IN + len(outs) == N_SEM
    wait(outs)


def _kernel(xt_hbm, w1_hbm, w2t_hbm, o_hbm, xv, w1v, w2v, w1t, hp, ov, xf, xb, wb, w2p, sems):
    step = pl.program_id(0)

    @pl.when(step == 0)
    def _():
        for g in _input_copies(xt_hbm, w1_hbm, w2t_hbm, xv, w1v, w2v, sems):
            for c in g:
                c.start()

    @pl.when(step == 1)
    def _():
        groups = _input_copies(xt_hbm, w1_hbm, w2t_hbm, xv, w1v, w2v, sems)
        _compute(groups, o_hbm, xv, w1v, w2v, w1t, hp, ov, xf, xb, wb, w2p, sems)


@jax.jit
def pallas_standalone__dense_activation_silu__prompt_kernel(
    x: jax.Array,
    w1: jax.Array,
    w2: jax.Array,
):
    assert x.shape == (1, S, D) and w1.shape == (D, F) and w2.shape == (F, D)
    xt = x.reshape(S, D).T
    w2t = w2.T
    out_t = pl.pallas_call(
        _kernel,
        grid=(2,),
        in_specs=[pl.BlockSpec(memory_space=pl.ANY)] * 3,
        out_specs=pl.BlockSpec(memory_space=pl.ANY),
        out_shape=jax.ShapeDtypeStruct((D, S), x.dtype),
        scratch_shapes=[
            pltpu.VMEM((D, S), jnp.bfloat16),
            pltpu.VMEM((D, F), jnp.bfloat16),
            pltpu.VMEM((D, F), jnp.bfloat16),
            pltpu.VMEM((F // 2, D), jnp.uint32),
            pltpu.VMEM((F, S), jnp.float32),
            pltpu.VMEM((D, S), jnp.bfloat16),
            pltpu.VMEM((64, S), jnp.float32),
            pltpu.VMEM((64, 4, 8, U), jnp.float32),
            pltpu.VMEM((64, G, 8, U), jnp.float32),
            pltpu.VMEM((D // 2, F), jnp.uint32),
            pltpu.SemaphoreType.DMA((N_SEM,)),
        ],
        compiler_params=pltpu.CompilerParams(
            dimension_semantics=("arbitrary",),
            vmem_limit_bytes=100 * 1024 * 1024,
            disable_semaphore_checks=True,
            disable_bounds_checks=True,
        ),
    )(xt, w1, w2t)
    return out_t.T.reshape(1, S, D)
```
